```python
import os as _os
_os.environ.setdefault("JAX_PLATFORMS", "cpu")
import jax
import jax.numpy as jnp

def _softmax(x, axis=-1):
    return jax.nn.softmax(x, axis=axis)
def _gelu(x):
    return jax.nn.gelu(x, approximate=True)
def _silu(x):
    return jax.nn.silu(x)
def _sigmoid(x):
    return jax.nn.sigmoid(x)
def _layernorm(x, axis=-1, eps=1e-5):
    m = jnp.mean(x, axis=axis, keepdims=True)
    v = jnp.var(x, axis=axis, keepdims=True)
    return (x - m) / jnp.sqrt(v + eps)
def _scatter_add(tgt, idx, src, axis=0):
    return tgt.at[idx].add(src)
def _segment_sum(src, seg, n):
    return jax.ops.segment_sum(src, seg, n)
class _Rng:
    def __init__(self, key):
        self._k = key
    def _next(self):
        self._k, sub = jax.random.split(self._k)
        return sub
    def normal(self, shape):
        return jax.random.normal(self._next(), shape, dtype=jnp.bfloat16)
    def randint(self, lo, hi, shape):
        return jax.random.randint(self._next(), shape, lo, hi, dtype=jnp.int32)
    def uniform(self, shape, lo=0.0, hi=1.0):
        return jax.random.uniform(self._next(), shape, jnp.bfloat16, lo, hi)
    def permutation(self, n):
        return jax.random.permutation(self._next(), n)


kernel_name = 'parallel_sum__ssm_conv_s5__geglu_ffn__prompt'

def setup_inputs():
    _rng = _Rng(jax.random.key(int.from_bytes(__import__("os").urandom(4), "little")))
    _w = (lambda a: (lambda t: t.astype(jnp.bfloat16) if jnp.issubdtype(t.dtype, jnp.floating) else t)(jnp.asarray(a)))
    def _A_setup():
        B, S, D = 1, 2048, 512
        P = D
        Lambda_re = -0.5 * jnp.exp((lambda *s: _rng.normal(s) * 0.8)(P))
        Lambda_im = (lambda *s: _rng.normal(s) * 0.8)(P) * 1.0
        B_re = (lambda *s: _rng.normal(s) * 0.8)(P, D) * (D ** -0.5)
        B_im = (lambda *s: _rng.normal(s) * 0.8)(P, D) * (D ** -0.5)
        C_re = (lambda *s: _rng.normal(s) * 0.8)(D, P) * (P ** -0.5)
        C_im = (lambda *s: _rng.normal(s) * 0.8)(D, P) * (P ** -0.5)
        log_dt = (lambda *s: _rng.normal(s) * 0.8)(P) * 0.3 - 2.0
        Dskip = (lambda *s: _rng.normal(s) * 0.8)(D)
        return {
            "x": _w((lambda *s: _rng.normal(s) * 0.05)(B, S, D)),
            "Lambda_re": _w(Lambda_re),
            "Lambda_im": _w(Lambda_im),
            "B_re": _w(B_re),
            "B_im": _w(B_im),
            "C_re": _w(C_re),
            "C_im": _w(C_im),
            "log_dt": _w(log_dt),
            "Dskip": _w(Dskip),
        }
    _A_in = _A_setup()

    def _B_setup():
        B, S, D, F = 1, 2048, 512, 1376
        return {
            "x": _w((lambda *s: _rng.normal(s) * 0.05)(B, S, D)),
            "w_gate": _w((lambda *s: _rng.normal(s) * 0.05)(D, F)),
            "w_up": _w((lambda *s: _rng.normal(s) * 0.05)(D, F)),
            "w_down": _w((lambda *s: _rng.normal(s) * 0.05)(F, D)),
        }
    _B_in = _B_setup()

    return {
        "A_x": _A_in["x"],
        "A_Lambda_re": _A_in["Lambda_re"],
        "A_Lambda_im": _A_in["Lambda_im"],
        "A_B_re": _A_in["B_re"],
        "A_B_im": _A_in["B_im"],
        "A_C_re": _A_in["C_re"],
        "A_C_im": _A_in["C_im"],
        "A_log_dt": _A_in["log_dt"],
        "A_Dskip": _A_in["Dskip"],
        "B_x": _B_in["x"],
        "B_w_gate": _B_in["w_gate"],
        "B_w_up": _B_in["w_up"],
        "B_w_down": _B_in["w_down"],
    }

def reference(A_x, A_Lambda_re, A_Lambda_im, A_B_re, A_B_im, A_C_re, A_C_im, A_log_dt, A_Dskip, B_x, B_w_gate, B_w_up, B_w_down):
    def _A_ref(x, Lambda_re, Lambda_im, B_re, B_im, C_re, C_im, log_dt, Dskip):
        Bsz, L, H = x.shape
        Lam = Lambda_re + 1j * Lambda_im
        Bmat = B_re + 1j * B_im
        Cmat = C_re + 1j * C_im
        dt = jnp.exp(log_dt)
        Lam_bar = jnp.exp(dt * Lam)
        B_bar = ((Lam_bar - 1.0) / Lam)[:, None] * Bmat
        Bu = jnp.einsum("bld,pd->blp", x + 0j, B_bar)
        h = jnp.zeros_like(Bu[:, 0, :])
        hs = []
        for t in range(L):
            h = Lam_bar[None, :] * h + Bu[:, t, :]
            hs.append(h)
        hseq = jnp.stack(hs, 1)
        y = 2.0 * jnp.einsum("blp,dp->bld", hseq, Cmat).real + x * Dskip[None, None, :]
        return y

    def _B_ref(x, w_gate, w_up, w_down):
        return (_gelu(x @ w_gate) * (x @ w_up)) @ w_down

    x = A_x
    xn = _layernorm(x, axis=-1)
    return x + _A_ref(xn, A_Lambda_re, A_Lambda_im, A_B_re, A_B_im, A_C_re, A_C_im, A_log_dt, A_Dskip) + _B_ref(xn, B_w_gate, B_w_up, B_w_down)
```

```python
import jax
import jax.numpy as jnp
import jax.experimental.pallas as pl
import jax.experimental.pallas.tpu as pltpu

S, D, P, F = 2048, 512, 512, 1376
FP = 1408
N2 = P + FP
KH = D // 2
KD = 640
SEG0, SEG, NL = 52, 68, 3
NT = NL + 1
SEGS = [SEG0] + [SEG] * NL
ROW0 = [0] + [8 * SEG0 + 8 * SEG * i for i in range(NL)]
assert 8 * sum(SEGS) == S
PORDER = (0, 1, 3, 2, 4, 5, 6)
EPS = 1e-5

f32, bf16, u32 = jnp.float32, jnp.bfloat16, jnp.uint32


def _up(n, m):
    return (n + m - 1) // m * m


def _cmul(ar, ai, br, bi):
    return ar * br - ai * bi, ar * bi + ai * br


def _cfma(ar, ai, br, bi, cr, ci):
    return (ar * br - ai * bi) + cr, (ar * bi + ai * br) + ci


def _nt(a, b):
    return jax.lax.dot_general(a, b, (((1,), (1,)), ((), ())), preferred_element_type=f32)


def _nn(a, b):
    return jnp.dot(a, b, preferred_element_type=f32)


def _lhs7(a11, a12, a21, a22):
    return [(a11 + a22).astype(bf16), (a21 + a22).astype(bf16), a11.astype(bf16), a22.astype(bf16),
            (a11 + a12).astype(bf16), (a21 - a11).astype(bf16), (a12 - a22).astype(bf16)]


def _rhs5(b11, b12, b21, b22):
    return [(b11 + b22).astype(bf16), (b12 - b22).astype(bf16), (b21 - b11).astype(bf16),
            (b11 + b12).astype(bf16), (b21 + b22).astype(bf16)]


def _combine(m):
    m1, m2, m3, m4, m5, m6, m7 = m
    return ((m1 + m4) - m5) + m7, m3 + m5, m2 + m4, ((m1 - m2) + m3) + m6


def _gelu_mul(g, u):
    c0 = 0.7978845608028654
    t = jnp.tanh(g * (c0 + (c0 * 0.044715) * (g * g)))
    h = (0.5 * g) * u
    return h + h * t


def _merge(a, b):
    out, i, j = [], 0, 0
    while i < len(a) or j < len(b):
        if j >= len(b) or (i < len(a) and i * len(b) <= j * len(a)):
            out.append(a[i])
            i += 1
        else:
            out.append(b[j])
            j += 1
    return out


class _Pins:
    def __init__(self, never):
        self.never = never

    @staticmethod
    def head(v):
        rows = 8 * (4 // v.dtype.itemsize)
        return pltpu.bitcast(v[:rows, :128], u32)

    def join(self, a, b):
        if a is None:
            return b
        if b is None:
            return a
        return jnp.where(self.never, a, b)

    def gate(self, v, tok):
        if tok is None:
            return v
        rows = 8 * (4 // v.dtype.itemsize)
        h = pltpu.bitcast(jnp.where(self.never, tok, self.head(v)), v.dtype)
        if v.shape[1] > 128:
            h = jnp.concatenate([h, v[:rows, 128:]], axis=1)
        if v.shape[0] > rows:
            h = jnp.concatenate([h, v[rows:]], axis=0)
        return h

    def gate_all(self, v, tok):
        if tok is None:
            return v
        w = pltpu.bitcast(v, u32)
        rep = (w.shape[0] // 8, w.shape[1] // 128)
        return pltpu.bitcast(jnp.where(jnp.tile(self.never, rep), jnp.tile(tok, rep), w), v.dtype)

    def interleave(self, mxu, side, lag, tail=0):
        n, m = len(mxu), len(side)
        slots = max(n - max(lag, tail), 1)
        k = 0
        done = {}
        for i, f in enumerate(mxu):
            res = f(done.get(i - lag - 1) if lag >= 0 else None)
            hi = m if i >= slots - 1 else (i + 1) * m // slots
            tok = None
            k0, nb = k, res.shape[0] // 8
            while k < hi:
                b = nb * (k - k0) // (hi - k0)
                t = side[k](pltpu.bitcast(res[8 * b:8 * b + 8, :128], u32))
                if lag >= 0:
                    tok = self.join(tok, t)
                k += 1
            done[i] = tok
        while k < m:
            side[k](None)
            k += 1


def _kernel(x_hbm, lre_hbm, lim_hbm, ldt_hbm, dsk_hbm,
            bre_hbm, bim_hbm, cre_hbm, cim_hbm, wg_hbm, wu_hbm, wd_hbm,
            o_hbm,
            x0_v, xl_v, lre_v, lim_v, ldt_v, dsk_v, w1_v, s1_v, cre_v, cim_v, sc_v, wd_v, sd_v, o0_v, ol_v,
            lhs_v, xb_v, res_v, cst_v, fen_v, sems):
    nsem = [0]

    def cp(src, dst):
        nsem[0] += 1
        return pltpu.make_async_copy(src, dst, sems.at[nsem[0] - 1])
    c_prm = [cp(s, d) for s, d in ((lre_hbm, lre_v), (lim_hbm, lim_v), (ldt_hbm, ldt_v))]
    c_dsk = cp(dsk_hbm, dsk_v)
    c_x = [[cp(x_hbm.at[pl.ds(ROW0[t], 8 * SEGS[t]), pl.ds(c * 128, 128)],
               (x0_v.at[c, pl.ds(0, 8 * SEG0)] if t == 0 else xl_v.at[t - 1, c, pl.ds(0, 8 * SEG)]))
            for c in range(4)] for t in range(NT)]
    c_bre = [cp(bre_hbm.at[pl.ds(r, P // 2)], w1_v.at[0, pl.ds(r, P // 2)]) for r in (0, P // 2)]
    c_bim = cp(bim_hbm, w1_v.at[1, pl.ds(0, P)])

    c_wg = cp(wg_hbm, w1_v.at[0, pl.ds(P, F)])
    c_wu = cp(wu_hbm, w1_v.at[1, pl.ds(P, F)])
    c_cre = cp(cre_hbm, cre_v)
    c_cim = cp(cim_hbm, cim_v)
    c_wd = cp(wd_hbm, wd_v.at[pl.ds(0, F)])
    c_fen = cp(x_hbm.at[pl.ds(0, 16), pl.ds(0, 128)], fen_v.at[1])
    c_fen2 = cp(x_hbm.at[pl.ds(0, 16), pl.ds(128, 128)], fen_v.at[2])
    k_out = nsem[0]

    def c_o(t, row0, seg, ov, c):
        return pltpu.make_async_copy(ov.at[c, pl.ds(0, 8 * seg)],
                                     o_hbm.at[pl.ds(row0, 8 * seg), pl.ds(c * 128, 128)], sems.at[k_out + 4 * t + c])

    for c in [c_dsk] + c_x[0] + c_bre + c_prm + [c_bim, c_wg, c_wu, c_cre, c_cim, c_wd] + c_x[1]:
        c.start()
    for t in range(2, NT):
        for c in c_x[t]:
            c.start()

    fen_v[0] = jnp.zeros((16, 128), bf16)
    zpad = jnp.zeros((FP - F, D), bf16)
    w1_v[0, pl.ds(P + F, FP - F), :] = zpad
    w1_v[1, pl.ds(P + F, FP - F), :] = zpad
    wd_v[pl.ds(F, FP - F), :] = zpad

    xu0_v = x0_v.bitcast(u32)
    xul_v = xl_v.bitcast(u32)

    c_dsk.wait()
    for c in c_x[0]:
        c.wait()
    dsk = dsk_v[...].astype(f32).reshape(1, D)
    pins = _Pins((pltpu.bitcast(jnp.broadcast_to(dsk[:, :128], (8, 128)), u32) & jnp.uint32(0xFFFF)) != 0)
    head, gate, gate_all, interleave = pins.head, pins.gate, pins.gate_all, pins.interleave
    cst = {}

    def load_x(tn, seg, i, tok):
        ev, od = [], []
        for jj in (2 * i, 2 * i + 1):
            rows = pl.ds(jj, 8, stride=seg // 2)
            w = [(xu0_v[c, rows, :] if tn is None else xul_v[tn, c, rows, :]) for c in range(4)]
            w = gate_all(jnp.concatenate(w, axis=1), tok)
            ev.append(pltpu.bitcast(w << 16, f32))
            od.append(pltpu.bitcast(w & jnp.uint32(0xFFFF0000), f32))
        return jnp.concatenate(ev + od, axis=0)

    def ln_group(tn, seg, slot, i):
        hm = 4 * seg

        def run(tok=None):
            x = load_x(tn, seg, i, tok)
            m = jnp.mean(x, axis=-1, keepdims=True)
            xc = x - m
            v = jnp.mean(xc * xc, axis=-1, keepdims=True)
            xn = xc * jax.lax.rsqrt(v + EPS)
            r = pl.ds(16 * i, 16)
            r2 = pl.ds(hm + 16 * i, 16)
            if tn is None:
                xb_v[r, :] = xn[:16].astype(bf16)
                z = xn[16:].astype(bf16)
                xb_v[r2, :] = z
            else:
                rs = x + xn * dsk
                res_v[slot, r, :] = rs[:16]
                res_v[slot, r2, :] = rs[16:]
                for k, z in enumerate(_lhs7(xn[:16, :KH], xn[:16, KH:], xn[16:, :KH], xn[16:, KH:])):
                    lhs_v[k, r, :] = z
            return head(z)
        return run

    def res0_group(i):
        def run(tok=None):
            x = load_x(None, SEG0, i, tok)
            for half in range(2):
                r = pl.ds(half * 4 * SEG0 + 16 * i, 16)
                rs = x[16 * half:16 * half + 16] + xb_v[r, :].astype(f32) * dsk
                res_v[0, r, :] = rs
            return head(rs)
        return run

    for i in range(SEG0 // 4):
        ln_group(None, SEG0, 0, i)()
    c_bre[0].wait()

    def params(tok=None):
        lre, lim, ldt = [jnp.broadcast_to(r[...].astype(f32).reshape(1, P), (8, P)) for r in (lre_v, lim_v, ldt_v)]
        ldt = gate_all(ldt, tok)
        dt = jnp.exp(ldt).astype(bf16).astype(f32)
        mag = jnp.exp(dt * lre)
        l1r = mag * jnp.cos(dt * lim)
        l1i = mag * jnp.sin(dt * lim)
        row = jax.lax.broadcasted_iota(jnp.int32, (8, P), 0)

        def cpow(n):
            rr, ri = None, None
            br, bi = l1r, l1i
            while n:
                if n & 1:
                    rr, ri = (br, bi) if rr is None else _cmul(rr, ri, br, bi)
                n >>= 1
                if n:
                    br, bi = _cmul(br, bi, br, bi)
            return rr, ri

        cst_v[0] = l1r
        cst_v[1] = l1i
        for n, seg in enumerate((SEG0, SEG)):
            a1 = cpow(seg)
            a2 = _cmul(*a1, *a1)
            a4 = _cmul(*a2, *a2)
            for k, (sh, a) in enumerate(((1, a1), (2, a2), (4, a4))):
                cst_v[2 + 6 * n + 2 * k] = jnp.where(row >= sh, a[0], 0.0)
                cst_v[3 + 6 * n + 2 * k] = jnp.where(row >= sh, a[1], 0.0)
        nr = l1r - 1.0
        ni = l1i
        big = jnp.abs(lre) >= jnp.abs(lim)
        ratio = jnp.where(big, lim / lre, lre / lim)
        den = jnp.where(big, lre + lim * ratio, lim + lre * ratio)
        gr = jnp.where(big, nr + ni * ratio, nr * ratio + ni) / den
        gi = jnp.where(big, ni - nr * ratio, ni * ratio - nr) / den
        cst['g'] = (2.0 * gr, 2.0 * gi)
        return pins.join(head(cst['g'][1]), head(a4[0]))

    def prep_c(q):
        def run(tok=None):
            gr, gi = cst['g']
            gr = gate_all(gr, tok)
            gi = gate_all(gi, tok)
            gr = jnp.concatenate([gr, gr], axis=0)
            gi = jnp.concatenate([gi, gi], axis=0)
            ngi = -gi
            v = []
            for half in range(2):
                rows = pl.ds(256 * half + 16 * q, 16)
                cre = cre_v[rows, :].astype(f32)
                cim = cim_v[rows, :].astype(f32)
                wr = cre * gr - cim * gi
                wi = cre * ngi - cim * gr
                cre_v[rows, :] = wr.astype(bf16)
                cim_v[rows, :] = wi.astype(bf16)
                v.append((wr, wi))
            for i, z in enumerate(_rhs5(v[0][0], v[1][0], v[0][1], v[1][1])):
                sc_v[i, pl.ds(16 * q, 16), :] = z
            return head(z)
        return run

    def prep_d(q):
        def run(tok=None):
            r1 = pl.ds(16 * q, 16)
            r2 = pl.ds(KD + 16 * q, 16)
            a = gate_all(wd_v[r1, :], tok).astype(f32)
            b = gate_all(wd_v[r2, :], tok).astype(f32)
            for i, z in enumerate(_rhs5(a[:, :256], a[:, 256:], b[:, :256], b[:, 256:])):
                sd_v[i, r1, :] = z
            return head(z)
        return run

    ch = {'re': ([(0, 0), (0, 128)], [(0, 256), (0, 384)], 0),
          'im': ([(1, 0), (1, 128)], [(1, 256), (1, 384)], 256)}
    for q in range(5):
        ch[q] = ([(0, P + 128 * q), (1, P + 128 * q)], [(0, P + KD + 128 * q), (1, P + KD + 128 * q)], 512 + 256 * q)
    ch[5] = ([(0, P + 2 * KD)], [(1, P + 2 * KD)], 512 + 256 * 5)

    def prep_1(name, k, r):
        n1, n2, base = ch[name]
        (h1, r1), (h2, r2) = n1[k], n2[k]

        def run(tok=None):
            a = gate_all(w1_v[h1, pl.ds(r1 + r, 16), :], tok).astype(f32)
            b = gate_all(w1_v[h2, pl.ds(r2 + r, 16), :], tok).astype(f32)
            for i, z in enumerate(_rhs5(a[:, :KH], b[:, :KH], a[:, KH:], b[:, KH:])):
                s1_v[i, pl.ds(base + 128 * k + r, 16), :] = z
            return head(z)
        return run

    def preps(name, ks):
        return [prep_1(name, k, r) for k in ks for r in range(0, 128, 16)]

    def stage1_plain(half, n, out):
        def run(tok=None):
            out[half, n] = _nt(gate(xb_v[...], tok), w1_v[half, pl.ds(128 * n, 128), :])
            return out[half, n]
        return run

    def stage1(name, out):
        n1, n2, base = ch[name]
        nr = 128 * len(n1)

        def plain(tiles, k0):
            parts = [w1_v[h, pl.ds(r, 128), pl.ds(k0, KH)] for h, r in tiles]
            return parts[0] if len(parts) == 1 else jnp.concatenate(parts, axis=0)
        srcs = [lambda: s1_v[0, pl.ds(base, nr), :], lambda: plain(n1, 0), lambda: s1_v[1, pl.ds(base, nr), :],
                lambda: s1_v[2, pl.ds(base, nr), :], lambda: plain(n2, KH), lambda: s1_v[3, pl.ds(base, nr), :],
                lambda: s1_v[4, pl.ds(base, nr), :]]
        m = [None] * 7

        def mk(i):
            def run(tok=None):
                m[i] = _nt(gate(lhs_v[i], tok), srcs[i]())
                if i == 6:
                    out['c'] = _combine(m)
                return m[i]
            return run
        return [mk(i) for i in range(7)]

    def scan_parts(seg, n, u, st, n1):
        loc = {}
        hr, hi = [], []

        def p1(j0, j1):
            def run(tok=None):
                lr, li = gate_all(cst_v[0], tok), cst_v[1]
                for j in range(j0, j1):
                    loc['e'] = u(0) if j == 0 else _cfma(lr, li, *loc['e'], *u(j))
                return head(loc['e'][0])
            return run

        def carry(tok=None):
            er, ei = loc['e']
            row = jax.lax.broadcasted_iota(jnp.int32, (8, P), 0)
            if st['f'] is None:
                cr = jnp.where(row == 0, 0.0, pltpu.roll(er, 1, 0))
                ci = jnp.where(row == 0, 0.0, pltpu.roll(ei, 1, 0))
            else:
                cr = pltpu.roll(jnp.where(row == 7, st['f'][0], er), 1, 0)
                ci = pltpu.roll(jnp.where(row == 7, st['f'][1], ei), 1, 0)
            for k, sh in enumerate((1, 2, 4)):
                sr = pltpu.roll(cr, sh, 0)
                si = pltpu.roll(ci, sh, 0)
                cr, ci = _cfma(cst_v[2 + 6 * n + 2 * k], cst_v[3 + 6 * n + 2 * k], sr, si, cr, ci)
            loc['c'] = (cr, ci)
            return head(cr)

        def p2(j0, j1):
            def run(tok=None):
                lr, li = gate_all(cst_v[0], tok), cst_v[1]
                for j in range(j0, j1):
                    loc['c'] = _cfma(lr, li, *loc['c'], *u(j))
                    hr.append(loc['c'][0])
                    hi.append(loc['c'][1])
                return head(loc['c'][0])
            return run

        def fin():
            st['f'] = loc['c']
            st['h'] = _lhs7(jnp.concatenate(hr[0::2], axis=0), jnp.concatenate(hi[0::2], axis=0),
                            jnp.concatenate(hr[1::2], axis=0), jnp.concatenate(hi[1::2], axis=0))

        b = [2 * ((seg // 2) * i // n1) for i in range(n1 + 1)]
        return [p1(b[i], b[i + 1]) for i in range(n1)] + [carry] + [p2(b[i], b[i + 1]) for i in range(n1)], fin

    def stage2(t, seg, row0, ov, slot, hc, zd, zl, side_c, side_d, nq):
        hm = 4 * seg
        wq = 256 // nq
        ftok = None
        for cq in range(nq):
            lo = cq * wq
            csrc = [lambda: sc_v[0, pl.ds(lo, wq), :], lambda: cre_v[pl.ds(lo, wq), :],
                    lambda: sc_v[1, pl.ds(lo, wq), :], lambda: sc_v[2, pl.ds(lo, wq), :],
                    lambda: cim_v[pl.ds(256 + lo, wq), :],
                    lambda: sc_v[3, pl.ds(lo, wq), :], lambda: sc_v[4, pl.ds(lo, wq), :]]
            dsrc = [lambda: sd_v[0, :, pl.ds(lo, wq)], lambda: wd_v[pl.ds(0, KD), pl.ds(lo, wq)],
                    lambda: sd_v[1, :, pl.ds(lo, wq)], lambda: sd_v[2, :, pl.ds(lo, wq)],
                    lambda: wd_v[pl.ds(KD, KD), pl.ds(256 + lo, wq)],
                    lambda: sd_v[3, :, pl.ds(lo, wq)], lambda: sd_v[4, :, pl.ds(lo, wq)]]
            mc = [None] * 7
            mm = [None] * 7
            yl = {}
            pend = {}
            early = side_c is None and cq == nq - 1

            def emit(rhalf, chalf, y):
                o = None
                for cc in range(wq // 128):
                    c = chalf * 2 + lo // 128 + cc
                    yc = chalf * wq + cc * 128
                    for jj in range(seg // 2):
                        r0 = rhalf * hm + 8 * jj
                        o = ((res_v[slot, pl.ds(r0, 8), pl.ds(128 * c, 128)] + yl['l'][r0:r0 + 8, yc:yc + 128])
                             + y[8 * jj:8 * jj + 8, cc * 128:cc * 128 + 128])
                        ov[c, pl.ds(2 * jj + rhalf, 8, stride=seg), :] = o
                return head(o)

            def after(n):
                need = (((0, 0), (0, 3, 4, 6), lambda: ((mm[0] + mm[3]) - mm[4]) + mm[6]),
                        ((0, 1), (2, 4), lambda: mm[2] + mm[4]),
                        ((1, 0), (1, 3), lambda: mm[1] + mm[3]),
                        ((1, 1), (0, 1, 2, 5), lambda: ((mm[0] - mm[1]) + mm[2]) + mm[5]))
                tok = None
                for key, req, fn in need:
                    if all(i in PORDER[:n] for i in req) and not all(i in PORDER[:n - 1] for i in req):
                        tok = pins.join(tok, emit(key[0], key[1], fn()))
                return tok

            def mkc(i):
                def run(tok=None):
                    mc[i] = _nt(gate(hc[i], tok), csrc[i]())
                    return mc[i]
                return run

            def mkd(i, n):
                def run(tok=None):
                    tok = pins.join(tok, pend.pop(n - 2, None))
                    mm[i] = mc[i] + _nn(gate(jnp.concatenate(zd[i], axis=1), tok), dsrc[i]())
                    pend[n] = after(n)
                    if early and n == 6:
                        for cc in range(wq // 128):
                            c_o(t, row0, seg, ov, 2 + lo // 128 + cc).start()
                        c_fen2.start()
                        pend[5] = pins.join(pend.pop(5, None), pltpu.bitcast(fen_v[t // 16, :, :], u32))
                    return mm[i]
                return run

            def mkl(tok=None):
                w = jnp.concatenate([wd_v[pl.ds(2 * KD, 128), pl.ds(lo, wq)],
                                     wd_v[pl.ds(2 * KD, 128), pl.ds(256 + lo, wq)]], axis=1)
                yl['l'] = _nn(gate(zl['z'], tok), w)
                return yl['l']

            if side_c is not None:
                interleave([mkc(i) for i in PORDER], side_c, lag=-1)
                interleave([mkl] + [mkd(i, n + 1) for n, i in enumerate(PORDER)], side_d, lag=-1)
            else:
                mx = []
                for n, i in enumerate(PORDER):
                    mx += [mkc(i), mkd(i, n + 1)] + ([mkl] if n == 0 else [])
                cut = [0] + ([len(side_d) * 7 // 10] if nq == 2 else []) + [len(side_d)]
                if ftok is not None:
                    f0 = mx[2]
                    mx[2] = (lambda tok=None, f0=f0, ft=ftok: f0(pins.join(tok, ft)))
                interleave(mx, side_d[cut[cq]:cut[cq + 1]], lag=4)
            for hf in range(1 if early else 2):
                for cc in range(wq // 128):
                    c_o(t, row0, seg, ov, hf * 2 + lo // 128 + cc).start()
            if side_c is None and cq == 0:
                c_fen.start()
                ftok = pltpu.bitcast(fen_v[t // 8], u32)

    st = {'f': None}
    hm = 4 * SEG0
    zd = [[None] * 5 for _ in range(7)]
    zl = {}
    o1 = {}
    gt = [(4 + q, 4 + q + 5) for q in range(5)] + [(14,)]

    for n in range(2):
        stage1_plain(0, n, o1)()
    for c in [c_bre[1]] + c_prm + [c_bim]:
        c.wait()
    interleave([stage1_plain(0, n, o1) for n in (2, 3)] + [stage1_plain(1, n, o1) for n in range(4)],
               preps('re', (0, 1)) + [params] + preps('im', (0, 1)), lag=0)
    c_wg.wait()

    def u0(j):
        r0 = (j % 2) * hm + 8 * (j // 2)
        return (jnp.concatenate([o1[0, n][r0:r0 + 8] for n in range(4)], axis=1),
                jnp.concatenate([o1[1, n][r0:r0 + 8] for n in range(4)], axis=1))
    sp, fin = scan_parts(SEG0, 0, u0, st, 2)
    gb = [stage1_plain(0, n, o1) for q in range(6) for n in gt[q]]
    interleave(gb[:7], [(lambda tok=None, f=f: f(None)) for f in sp], lag=0)
    interleave(gb[7:], [f for q in range(5) for f in preps(q, (0,))] + [res0_group(i) for i in range(SEG0 // 4)], lag=0)
    for c in (c_wu, c_cre, c_cim):
        c.wait()

    def up_act(f, q):
        def run(tok=None):
            r = f(tok)
            a = _gelu_mul(jnp.concatenate([o1[0, n] for n in gt[q]], axis=1),
                          jnp.concatenate([o1[1, n] for n in gt[q]], axis=1))
            if q == 5:
                zl['z'] = a.astype(bf16)
            else:
                for i, z in enumerate(_lhs7(a[:hm, :128], a[:hm, 128:], a[hm:, :128], a[hm:, 128:])):
                    zd[i][q] = z
            return r
        return run
    mx = []
    for q in range(6):
        fs = [stage1_plain(1, n, o1) for n in gt[q]]
        mx += fs[:-1] + [up_act(fs[-1], q)]
    interleave(mx, [prep_c(q) for q in range(16)], lag=0)
    for c in [c_wd] + c_x[1]:
        c.wait()
    fin()
    p1s = [f for q in range(5) for f in preps(q, (1,))] + preps(5, (0,))
    ln = [ln_group(0, SEG, 1, i) for i in range(SEG // 4)]
    stage2(0, SEG0, 0, o0_v, 0, st['h'], zd, zl,
           [prep_d(q) for q in range(KD // 16)] + p1s[:16], _merge(ln, p1s[16:]), 1)
    for t in range(2, NT):
        for c in c_x[t]:
            c.wait()

    def body(t, carry):
        st = {'f': carry}
        row0 = pl.multiple_of(ROW0[1] + (t - 1) * (8 * SEG), 8)
        tn = jnp.minimum(t, NL - 1)
        slot = t % 2
        are, aim = {}, {}
        for f in stage1('re', are) + stage1('im', aim):
            f()

        def u(j):
            blk = slice(8 * (j // 2), 8 * (j // 2) + 8)
            o = 2 * (j % 2)
            return (jnp.concatenate([are['c'][o][blk], are['c'][o + 1][blk]], axis=1),
                    jnp.concatenate([aim['c'][o][blk], aim['c'][o + 1][blk]], axis=1))
        zd = [[None] * 5 for _ in range(7)]
        zl = {}
        gos = [{} for _ in range(6)]

        def with_act(f, q):
            def run(tok=None):
                r = f(tok)
                c11, c12, c21, c22 = gos[q]['c']
                if q < 5:
                    for i, z in enumerate(_lhs7(*[_gelu_mul(z[:, :128], z[:, 128:]) for z in (c11, c12, c21, c22)])):
                        zd[i][q] = z
                else:
                    zl['z'] = jnp.concatenate([_gelu_mul(c11, c12), _gelu_mul(c21, c22)], axis=0).astype(bf16)
                return r
            return run
        mx = []
        for q in range(6):
            fs = stage1(q, gos[q])
            mx += fs[:-1] + [with_act(fs[-1], q)]
        sp, fin = scan_parts(SEG, 1, u, st, 4)
        interleave(mx[:14], sp, lag=4)
        for f in mx[14:]:
            f()
        fin()
        stage2(t, SEG, row0, ol_v.at[t - 1], slot, st['h'], zd, zl, None,
               [ln_group(tn, SEG, 1 - slot, i) for i in range(SEG // 4)], 2)
        c_fen.wait()
        c_fen2.wait()
        return st['f']

    jax.lax.fori_loop(1, NT, body, st['f'])
    for t in range(NT):
        for c in range(4):
            c_o(t, ROW0[t], SEGS[t], o0_v if t == 0 else ol_v.at[t - 1], c).wait()


N_SEMS = 4 + 4 * NT + 2 + 1 + 1 + 4 + 2 + 4 * NT


@jax.jit
def pallas_parallel_sum__ssm_conv_s5__geglu_ffn__prompt_kernel(
    A_x: jax.Array,
    A_Lambda_re: jax.Array,
    A_Lambda_im: jax.Array,
    A_B_re: jax.Array,
    A_B_im: jax.Array,
    A_C_re: jax.Array,
    A_C_im: jax.Array,
    A_log_dt: jax.Array,
    A_Dskip: jax.Array,
    B_x: jax.Array,
    B_w_gate: jax.Array,
    B_w_up: jax.Array,
    B_w_down: jax.Array,
):
    del B_x
    hbm = pl.BlockSpec(memory_space=pltpu.HBM)
    vec = pltpu.VMEM((P,), bf16)
    out = pl.pallas_call(
        _kernel,
        in_specs=[hbm] * 12,
        out_specs=hbm,
        out_shape=jax.ShapeDtypeStruct((S, D), f32),
        scratch_shapes=[
            pltpu.VMEM((4, _up(9 * SEG0, 16), 128), bf16), pltpu.VMEM((NL, 4, _up(9 * SEG, 16), 128), bf16),
            vec, vec, vec, vec,
            pltpu.VMEM((2, N2, D), bf16), pltpu.VMEM((5, N2, KH), bf16),
            pltpu.VMEM((D, P), bf16), pltpu.VMEM((D, P), bf16), pltpu.VMEM((5, D // 2, P), bf16),
            pltpu.VMEM((FP, D), bf16), pltpu.VMEM((5, KD, D // 2), bf16),
            pltpu.VMEM((4, _up(9 * SEG0, 8), 128), f32), pltpu.VMEM((NL, 4, _up(9 * SEG, 8), 128), f32),
            pltpu.VMEM((7, 4 * SEG, KH), bf16), pltpu.VMEM((8 * SEG0, D), bf16),
            pltpu.VMEM((2, 8 * max(SEG0, SEG), D), f32),
            pltpu.VMEM((14, 8, P), f32),
            pltpu.VMEM((3, 16, 128), bf16),
            pltpu.SemaphoreType.DMA((N_SEMS,)),
        ],
        compiler_params=pltpu.CompilerParams(
            vmem_limit_bytes=100 * 1024 * 1024,
            disable_semaphore_checks=True,
            disable_bounds_checks=True,
        ),
    )(A_x.reshape(S, D), A_Lambda_re, A_Lambda_im, A_log_dt, A_Dskip,
      A_B_re, A_B_im, A_C_re, A_C_im, B_w_gate.T, B_w_up.T, B_w_down)
    return out.reshape(1, S, D)
```
